```python
import jax
import jax.numpy as jnp

def _softmax(x, axis=-1):
    return jax.nn.softmax(x, axis=axis)
def _gelu(x):
    return jax.nn.gelu(x, approximate=True)
def _silu(x):
    return jax.nn.silu(x)
def _sigmoid(x):
    return jax.nn.sigmoid(x)
def _layernorm(x, axis=-1, eps=1e-5):
    m = jnp.mean(x, axis=axis, keepdims=True)
    v = jnp.var(x, axis=axis, keepdims=True)
    return (x - m) / jnp.sqrt(v + eps)
def _scatter_add(tgt, idx, src, axis=0):
    return tgt.at[idx].add(src)
def _segment_sum(src, seg, n):
    return jax.ops.segment_sum(src, seg, n)
class _Rng:
    def __init__(self, key):
        self._k = key
    def _next(self):
        self._k, sub = jax.random.split(self._k)
        return sub
    def normal(self, shape):
        return jax.random.normal(self._next(), shape, dtype=jnp.bfloat16)
    def randint(self, lo, hi, shape):
        return jax.random.randint(self._next(), shape, lo, hi, dtype=jnp.int32)
    def uniform(self, shape, lo=0.0, hi=1.0):
        return jax.random.uniform(self._next(), shape, jnp.bfloat16, lo, hi)
    def permutation(self, n):
        return jax.random.permutation(self._next(), n)


kernel_name = 'gated_mix__sliding_block_cached__dense_activation_gelu__decode'

def setup_inputs():
    _rng = _Rng(jax.random.key(int.from_bytes(__import__("os").urandom(4), "little")))
    _w = (lambda a: (lambda t: t.astype(jnp.bfloat16) if jnp.issubdtype(t.dtype, jnp.floating) else t)(jnp.asarray(a)))
    def _A_setup():
        B, Sq, D = 1, 1, 640
        Hq, Hkv, Sk, Dh = 32, 32, 32768, 192
        assert Hq % Hkv == 0, (Hq, Hkv)
        return {
            "x": _w((lambda *s: _rng.normal(s) * 0.05)(B, Sq, D)),
            "k_cache": _w((lambda *s: _rng.normal(s) * 0.05)(B, Hkv, Sk, Dh)),
            "v_cache": _w((lambda *s: _rng.normal(s) * 0.05)(B, Hkv, Sk, Dh)),
            "wq": _w((lambda *s: _rng.normal(s) * 0.05)(D, Hq * Dh) * (D ** -0.5)),
            "wo": _w((lambda *s: _rng.normal(s) * 0.05)(Hq * Dh, D) * ((Hq * Dh) ** -0.5)),
        }
    _A_in = _A_setup()

    def _B_setup():
        B, S, D, F = 1, 1, 640, 1536
        return {
            "x": _w((lambda *s: _rng.normal(s) * 0.05)(B, S, D)),
            "w1": _w((lambda *s: _rng.normal(s) * 0.05)(D, F) * (D ** -0.5)),
            "b1": _w((lambda *s: _rng.normal(s) * 0.05)(F) * 0.01),
            "w2": _w((lambda *s: _rng.normal(s) * 0.05)(F, D) * (F ** -0.5)),
            "b2": _w((lambda *s: _rng.normal(s) * 0.05)(D) * 0.01),
        }
    _B_in = _B_setup()

    return {
        "A_x": _A_in["x"],
        "A_k_cache": _A_in["k_cache"],
        "A_v_cache": _A_in["v_cache"],
        "A_wq": _A_in["wq"],
        "A_wo": _A_in["wo"],
        "B_x": _B_in["x"],
        "B_w1": _B_in["w1"],
        "B_b1": _B_in["b1"],
        "B_w2": _B_in["w2"],
        "B_b2": _B_in["b2"],
        "gate_w": _w((lambda *s: _rng.normal(s) * 0.05)(640)),
    }

def reference(A_x, A_k_cache, A_v_cache, A_wq, A_wo, B_x, B_w1, B_b1, B_w2, B_b2, gate_w):
    def _A_ref(x, k_cache, v_cache, wq, wo):
        B, Sq, D = x.shape
        Hq, Dh = 32, 192
        Hkv, Sk = k_cache.shape[1], k_cache.shape[2]
        W = min(4096, max(256, Sk // 4))
        rep = Hq // Hkv
        q = (lambda x, *d: x.transpose(*d))((x @ wq).reshape(B, Sq, Hq, Dh), 0, 2, 1, 3)
        k = jnp.repeat(k_cache[:, :, Sk - W:, :], rep, axis=1)
        v = jnp.repeat(v_cache[:, :, Sk - W:, :], rep, axis=1)
        scores = jnp.einsum("bhqd,bhkd->bhqk", q, k) * (Dh ** -0.5)
        p = _softmax(scores, axis=-1)
        o = jnp.einsum("bhqk,bhkd->bhqd", p, v)
        return (lambda x, *d: x.transpose(*d))(o, 0, 2, 1, 3).reshape(B, Sq, Hq * Dh) @ wo

    def _B_ref(x, w1, b1, w2, b2):
        h = jnp.einsum("bsd,df->bsf", x, w1) + b1
        h = _gelu(h)
        return jnp.einsum("bsf,fd->bsd", h, w2) + b2

    x = A_x
    g = _sigmoid((x * gate_w).sum(-1, keepdims=True))
    a = _A_ref(x, A_k_cache, A_v_cache, A_wq, A_wo)
    b = _B_ref(x, B_w1, B_b1, B_w2, B_b2)
    return g * a + (1 - g) * b
```

```python
import functools

import jax
import jax.numpy as jnp
from jax import lax
import jax.experimental.pallas as pl
import jax.experimental.pallas.tpu as pltpu

F32 = jnp.float32
BF16 = jnp.bfloat16

HQ = 32
DH = 192
M = 16
RG = 8
AHEAD = 2
NB = AHEAD + 1
KV_SPLIT = 1792
WQ_ROWS = 128
WO_HEADS = 4


def _kernel(x_hbm, kt_hbm, vt_hbm, wq_hbm, wo_hbm, w1_hbm, b1_hbm, w2_hbm, b2_hbm, gw_hbm,
            out_ref,
            x_v, gw_v, b1_v, b2_v, wq_v, wo_v, w1_v, w2_v, kbuf, vbuf, qacc, qh, oh,
            small_sem, wq_sem, wo_sem, w1_sem, w2_sem, k_sem, v_sem,
            *, sk, win):
    d_model = wq_v.shape[0]
    d_ff = w1_v.shape[1]
    c0 = sk - win
    n_wq = d_model // WQ_ROWS
    n_wo = HQ // WO_HEADS

    def copy(src, dst, sem, prio):
        pltpu.make_async_copy(src, dst, sem).start(priority=prio)

    def wait_all(buf, sem):
        pltpu.make_async_copy(buf, buf, sem).wait()

    def issue_kv(src_hbm, buf, sem, h):
        slot = h % NB

        def body(g, c):
            r_src = pl.multiple_of(h * DH + g * RG, RG)
            r_dst = pl.multiple_of(g * RG, RG)
            copy(src_hbm.at[pl.ds(r_src, RG), pl.ds(c0, KV_SPLIT)],
                 buf.at[slot, pl.ds(r_dst, RG), pl.ds(0, KV_SPLIT)], sem.at[slot], 0)
            copy(src_hbm.at[pl.ds(r_src, RG), pl.ds(c0 + KV_SPLIT, win - KV_SPLIT)],
                 buf.at[slot, pl.ds(r_dst, RG), pl.ds(KV_SPLIT, win - KV_SPLIT)], sem.at[slot], 1)
            return c
        lax.fori_loop(0, DH // RG, body, 0)

    def issue_wq(j):
        cuts = (0, 1792, 3840, 6144)

        def body(g, c):
            for u in range(2):
                r = pl.multiple_of(j * WQ_ROWS + (2 * g + u) * RG, RG)
                for t in range(3):
                    a, b = cuts[t], cuts[t + 1]
                    copy(wq_hbm.at[pl.ds(r, RG), pl.ds(a, b - a)],
                         wq_v.at[pl.ds(r, RG), pl.ds(a, b - a)], wq_sem.at[j], (u + t) % 2)
            return c
        lax.fori_loop(0, WQ_ROWS // RG // 2, body, 0)

    def issue_rows(src_hbm, dst, sem, row0, nrows, step):
        def body(g, c):
            for u in range(2):
                r = pl.multiple_of(row0 + (2 * g + u) * step, RG)
                copy(src_hbm.at[pl.ds(r, step)], dst.at[pl.ds(r, step)], sem, u)
            return c
        lax.fori_loop(0, nrows // step // 2, body, 0)

    def issue_wo(j):
        issue_rows(wo_hbm, wo_v, wo_sem.at[j], j * WO_HEADS * DH, WO_HEADS * DH, 24)

    small = [(x_hbm, x_v), (gw_hbm, gw_v), (b1_hbm, b1_v), (b2_hbm, b2_v)]
    for i, (s, d) in enumerate(small):
        copy(s, d, small_sem.at[i], 0)
    for j in range(n_wq):
        issue_wq(j)
    issue_rows(w1_hbm, w1_v, w1_sem, 0, d_model, RG)
    for i, (s, d) in enumerate(small):
        pltpu.make_async_copy(s, d, small_sem.at[i]).wait()

    x = x_v[0]
    xm = jnp.broadcast_to(x, (M, d_model))

    def q_part(j):
        wait_all(wq_v.at[pl.ds(j * WQ_ROWS, WQ_ROWS)], wq_sem.at[j])
        part = jnp.dot(xm[:, j * WQ_ROWS:(j + 1) * WQ_ROWS], wq_v[j * WQ_ROWS:(j + 1) * WQ_ROWS, :],
                       preferred_element_type=F32)
        if j == 0:
            qacc[...] = part
        else:
            qacc[...] += part

    q_part(0)
    q_part(1)
    q_part(2)
    issue_kv(kt_hbm, kbuf, k_sem, 0)
    q_part(3)
    issue_kv(vt_hbm, vbuf, v_sem, 0)
    q_part(4)
    for h in range(HQ):
        qh[h] = qacc[:, h * DH:(h + 1) * DH].astype(BF16)
    issue_kv(kt_hbm, kbuf, k_sem, 1)
    wait_all(w1_v, w1_sem)
    hid = jnp.dot(xm, w1_v[...], preferred_element_type=F32) + b1_v[...].astype(F32).reshape(1, d_ff)
    hid = jax.nn.gelu(hid, approximate=True).astype(BF16)
    issue_kv(vt_hbm, vbuf, v_sem, 1)

    scale = DH ** -0.5

    def head(h, issue_k, issue_v):
        slot = h % NB
        issue_k()
        wait_all(kbuf.at[slot], k_sem.at[slot])
        s = jnp.dot(qh[h], kbuf[slot], preferred_element_type=F32)[0:8] * scale
        m = jnp.max(s, axis=1, keepdims=True)
        p = jnp.exp(s - m)
        l = jnp.sum(p, axis=1, keepdims=True)
        pb = p.astype(BF16)
        issue_v()
        wait_all(vbuf.at[slot], v_sem.at[slot])
        o = lax.dot_general(pb, vbuf[slot], (((1,), (1,)), ((), ())), preferred_element_type=F32)
        oh[h] = (o / l).astype(BF16)

    def loop_body(h, c):
        head(h, lambda: issue_kv(kt_hbm, kbuf, k_sem, h + AHEAD),
             lambda: issue_kv(vt_hbm, vbuf, v_sem, h + AHEAD))
        return c
    lax.fori_loop(0, HQ - AHEAD, loop_body, 0)

    head(HQ - 2, lambda: issue_rows(w2_hbm, w2_v, w2_sem, 0, d_ff, 24), lambda: issue_wo(0))
    head(HQ - 1, lambda: issue_wo(1), lambda: issue_wo(2))

    issue_wo(3)
    wait_all(w2_v, w2_sem)
    ffn = jnp.dot(hid, w2_v[...], preferred_element_type=F32)[0:1] + b2_v[...].astype(F32).reshape(1, d_model)
    gate = jax.nn.sigmoid(jnp.sum(x.astype(F32) * gw_v[...].astype(F32).reshape(1, d_model),
                                  axis=1, keepdims=True))

    acc = jnp.zeros((8, d_model), F32)
    for j in range(n_wo):
        if j + 4 < n_wo:
            issue_wo(j + 4)
        wait_all(wo_v.at[pl.ds(j * WO_HEADS * DH, WO_HEADS * DH)], wo_sem.at[j])
        for hh in range(WO_HEADS):
            h = j * WO_HEADS + hh
            acc = acc + jnp.dot(oh[h], wo_v[h * DH:(h + 1) * DH, :], preferred_element_type=F32)
    res = gate * acc[0:1] + (1.0 - gate) * ffn
    out_ref[0] = res.astype(out_ref.dtype)


@jax.jit
def pallas_gated_mix__sliding_block_cached__dense_activation_gelu__decode_kernel(
    A_x: jax.Array,
    A_k_cache: jax.Array,
    A_v_cache: jax.Array,
    A_wq: jax.Array,
    A_wo: jax.Array,
    B_x: jax.Array,
    B_w1: jax.Array,
    B_b1: jax.Array,
    B_w2: jax.Array,
    B_b2: jax.Array,
    gate_w: jax.Array,
):
    del B_x
    b, sq, d_model = A_x.shape
    _, hkv, sk, dh = A_k_cache.shape
    assert (b, sq, hkv, dh) == (1, 1, HQ, DH)
    d_ff = B_w1.shape[1]
    win = min(4096, max(256, sk // 4))
    kt = jnp.swapaxes(A_k_cache, 2, 3).reshape(HQ * DH, sk)
    vt = jnp.swapaxes(A_v_cache, 2, 3).reshape(HQ * DH, sk)

    any_spec = pl.BlockSpec(memory_space=pl.ANY)
    dma = pltpu.SemaphoreType.DMA
    return pl.pallas_call(
        functools.partial(_kernel, sk=sk, win=win),
        out_shape=jax.ShapeDtypeStruct((b, sq, d_model), A_x.dtype),
        in_specs=[any_spec] * 10,
        out_specs=pl.BlockSpec(memory_space=pltpu.VMEM),
        scratch_shapes=[
            pltpu.VMEM(A_x.shape, BF16),
            pltpu.VMEM(gate_w.shape, BF16),
            pltpu.VMEM(B_b1.shape, BF16),
            pltpu.VMEM(B_b2.shape, BF16),
            pltpu.VMEM(A_wq.shape, BF16),
            pltpu.VMEM(A_wo.shape, BF16),
            pltpu.VMEM(B_w1.shape, BF16),
            pltpu.VMEM(B_w2.shape, BF16),
            pltpu.VMEM((NB, DH, win), BF16),
            pltpu.VMEM((NB, DH, win), BF16),
            pltpu.VMEM((M, HQ * DH), F32),
            pltpu.VMEM((HQ, M, DH), BF16),
            pltpu.VMEM((HQ, 8, DH), BF16),
            dma((4,)), dma((d_model // WQ_ROWS,)), dma((HQ // WO_HEADS,)), dma, dma,
            dma((NB,)), dma((NB,)),
        ],
        compiler_params=pltpu.CompilerParams(
            vmem_limit_bytes=64 * 1024 * 1024,
            disable_bounds_checks=True,
        ),
    )(A_x, kt, vt, A_wq, A_wo, B_w1, B_b1, B_w2, B_b2, gate_w)
```

```python
import functools

import jax
import jax.numpy as jnp
from jax import lax
import jax.experimental.pallas as pl
import jax.experimental.pallas.tpu as pltpu

F32 = jnp.float32
BF16 = jnp.bfloat16

HQ = 32
DH = 192
M = 16
RG = 8
AHEAD = 2
NB = 4
KV_SPLIT = 1792
WQ_CUT = (0, 1792, 3840, 6144)
WO_CUT = (0, 3, 6, 9, 12, 16)
W2_ROWS = 32
W2_LAST = 256


def _kernel(x_hbm, kt_hbm, vt_hbm, wq_hbm, wo_hbm, w1_hbm, b1_hbm, w2_hbm, b2_hbm, gw_hbm,
            out_ref,
            x_v, gw_v, b1_v, b2_v, wq_v, wo_v, w1_v, w2_v, kbuf, vbuf, qh,
            small_sem, wq_sem, wo_sem, w1_sem, w2_sem, k_sem, v_sem,
            *, sk, win):
    d_model = wq_v.shape[0]
    d_ff = w1_v.shape[1]
    c0 = sk - win

    def copy(src, dst, sem, prio):
        pltpu.make_async_copy(src, dst, sem).start(priority=prio)

    def wait_all(buf, sem):
        pltpu.make_async_copy(buf, buf, sem).wait()

    def rows(src_hbm, dst, sem, r, n, prio):
        r = pl.multiple_of(r, RG)
        copy(src_hbm.at[pl.ds(r, n)], dst.at[pl.ds(r, n)], sem, prio)

    def issue_kv(src_hbm, buf, sem, h):
        slot = h & (NB - 1)

        def body(g, c):
            r_src = pl.multiple_of(h * DH + g * RG, RG)
            r_dst = pl.multiple_of(g * RG, RG)
            copy(src_hbm.at[pl.ds(r_src, RG), pl.ds(c0, KV_SPLIT)],
                 buf.at[slot, pl.ds(r_dst, RG), pl.ds(0, KV_SPLIT)], sem.at[slot], 0)
            copy(src_hbm.at[pl.ds(r_src, RG), pl.ds(c0 + KV_SPLIT, win - KV_SPLIT)],
                 buf.at[slot, pl.ds(r_dst, RG), pl.ds(KV_SPLIT, win - KV_SPLIT)], sem.at[slot], 1)
            return c
        lax.fori_loop(0, DH // RG, body, 0)

    def w1_pair(p):
        rows(w1_hbm, w1_v, w1_sem, p * RG, RG, 0)
        rows(w1_hbm, w1_v, w1_sem, d_model // 2 + p * RG, RG, 1)

    def weights_pass(a, c):
        p0 = (5 * a) >> 1
        for n in range(15):
            j = (n - a) & 15
            r = pl.multiple_of(j * 40 + (n // 3) * RG, RG)
            ca, cb = WQ_CUT[n % 3], WQ_CUT[n % 3 + 1]
            copy(wq_hbm.at[pl.ds(r, RG), pl.ds(ca, cb - ca)],
                 wq_v.at[pl.ds(r, RG), pl.ds(ca, cb - ca)], wq_sem, 0)
            ra, rb = WO_CUT[n % 5], WO_CUT[n % 5 + 1]
            rows(wo_hbm, wo_v, wo_sem, j * 384 + (n // 5) * 128 + ra * RG, (rb - ra) * RG, 1)
            if n == 2:
                w1_pair(p0)
            if n == 8:
                w1_pair(p0 + 1)
            if n == 13:
                @pl.when((a & 1) == 1)
                def _():
                    w1_pair(p0 + 2)
        return c

    half = d_ff // 2
    w2_cut = d_ff - W2_LAST

    def issue_w2():
        def body(j, c):
            r = j * W2_ROWS
            rows(w2_hbm, w2_v, w2_sem.at[0], r, W2_ROWS, 0)
            last = (half + r >= w2_cut).astype(jnp.int32)
            rows(w2_hbm, w2_v, w2_sem.at[last], half + r, W2_ROWS, 1)
            return c
        lax.fori_loop(0, half // W2_ROWS, body, 0)

    lax.fori_loop(0, 16, weights_pass, 0)
    small = [(x_hbm, x_v), (gw_hbm, gw_v), (b1_hbm, b1_v), (b2_hbm, b2_v)]
    for i, (s, d) in enumerate(small):
        copy(s, d, small_sem.at[i], 0)
    issue_kv(kt_hbm, kbuf, k_sem, 0)
    issue_kv(vt_hbm, vbuf, v_sem, 0)
    for i, (s, d) in enumerate(small):
        pltpu.make_async_copy(s, d, small_sem.at[i]).wait()

    x = x_v[0]
    xm = jnp.broadcast_to(x, (M, d_model))

    def q_part(h0, h1):
        q = jnp.dot(xm, wq_v[:, h0 * DH:h1 * DH], preferred_element_type=F32).astype(BF16)
        for h in range(h0, h1):
            qh[h] = q[:, (h - h0) * DH:(h - h0 + 1) * DH]

    wait_all(wq_v, wq_sem)
    q_part(0, HQ // 2)
    issue_kv(kt_hbm, kbuf, k_sem, 1)
    q_part(HQ // 2, HQ)
    issue_kv(vt_hbm, vbuf, v_sem, 1)
    wait_all(w1_v, w1_sem)
    hid = jnp.dot(xm, w1_v[...], preferred_element_type=F32) + b1_v[...].astype(F32).reshape(1, d_ff)
    hid = jax.nn.gelu(hid[0:8], approximate=True).astype(BF16)
    gate = jax.nn.sigmoid(jnp.sum(x.astype(F32) * gw_v[...].astype(F32).reshape(1, d_model),
                                  axis=1, keepdims=True))
    b2 = b2_v[...].astype(F32).reshape(1, d_model)
    wait_all(wo_v, wo_sem)

    scale = DH ** -0.5

    def head(h, acc):
        slot = h & (NB - 1)

        @pl.when(h < HQ - AHEAD)
        def _():
            issue_kv(kt_hbm, kbuf, k_sem, h + AHEAD)

        @pl.when(h == HQ - AHEAD)
        def _():
            issue_w2()

        wait_all(kbuf.at[slot], k_sem.at[slot])
        s = jnp.dot(qh[h], kbuf[slot], preferred_element_type=F32)[0:8] * scale
        m = jnp.max(s, axis=1, keepdims=True)
        p = jnp.exp(s - m)
        inv_l = 1.0 / jnp.sum(p, axis=1, keepdims=True)
        pb = p.astype(BF16)

        @pl.when(h < HQ - AHEAD)
        def _():
            issue_kv(vt_hbm, vbuf, v_sem, h + AHEAD)

        wait_all(vbuf.at[slot], v_sem.at[slot])
        o = lax.dot_general(pb, vbuf[slot], (((1,), (1,)), ((), ())), preferred_element_type=F32)
        o = (o * inv_l).astype(BF16)
        r = pl.multiple_of(h * DH, 16)
        return acc + jnp.dot(o, wo_v[pl.ds(r, DH), :], preferred_element_type=F32)

    attn = lax.fori_loop(0, HQ, head, jnp.zeros((8, d_model), F32))

    res = gate * attn[0:1] + (1.0 - gate) * b2
    for st, (lo, hi) in enumerate(((0, w2_cut), (w2_cut, d_ff))):
        wait_all(w2_v.at[pl.ds(lo, hi - lo)], w2_sem.at[st])
        res = res + (1.0 - gate) * jnp.dot(hid[:, lo:hi], w2_v[lo:hi, :],
                                           preferred_element_type=F32)[0:1]
    out_ref[0] = res.astype(out_ref.dtype)


@jax.jit
def pallas_gated_mix__sliding_block_cached__dense_activation_gelu__decode_kernel(
    A_x: jax.Array,
    A_k_cache: jax.Array,
    A_v_cache: jax.Array,
    A_wq: jax.Array,
    A_wo: jax.Array,
    B_x: jax.Array,
    B_w1: jax.Array,
    B_b1: jax.Array,
    B_w2: jax.Array,
    B_b2: jax.Array,
    gate_w: jax.Array,
):
    del B_x
    b, sq, d_model = A_x.shape
    _, hkv, sk, dh = A_k_cache.shape
    win = min(4096, max(256, sk // 4))
    assert (b, sq, d_model, hkv, dh, win) == (1, 1, 640, HQ, DH, 4096)
    assert B_w1.shape == (d_model, 1536)
    kt = jnp.swapaxes(A_k_cache, 2, 3).reshape(HQ * DH, sk)
    vt = jnp.swapaxes(A_v_cache, 2, 3).reshape(HQ * DH, sk)

    any_spec = pl.BlockSpec(memory_space=pl.ANY)
    dma = pltpu.SemaphoreType.DMA
    return pl.pallas_call(
        functools.partial(_kernel, sk=sk, win=win),
        out_shape=jax.ShapeDtypeStruct((b, sq, d_model), A_x.dtype),
        in_specs=[any_spec] * 10,
        out_specs=pl.BlockSpec(memory_space=pltpu.VMEM),
        scratch_shapes=[
            pltpu.VMEM(A_x.shape, BF16),
            pltpu.VMEM(gate_w.shape, BF16),
            pltpu.VMEM(B_b1.shape, BF16),
            pltpu.VMEM(B_b2.shape, BF16),
            pltpu.VMEM(A_wq.shape, BF16),
            pltpu.VMEM(A_wo.shape, BF16),
            pltpu.VMEM(B_w1.shape, BF16),
            pltpu.VMEM(B_w2.shape, BF16),
            pltpu.VMEM((NB, DH, win), BF16),
            pltpu.VMEM((NB, DH, win), BF16),
            pltpu.VMEM((HQ, M, DH), BF16),
            dma((4,)), dma, dma, dma, dma((2,)), dma((NB,)), dma((NB,)),
        ],
        compiler_params=pltpu.CompilerParams(
            vmem_limit_bytes=64 * 1024 * 1024,
            disable_bounds_checks=True,
            disable_semaphore_checks=True,
        ),
    )(A_x, kt, vt, A_wq, A_wo, B_w1, B_b1, B_w2, B_b2, gate_w)
```

```python
import functools

import jax
import jax.numpy as jnp
from jax import lax
import jax.experimental.pallas as pl
import jax.experimental.pallas.tpu as pltpu

F32 = jnp.float32
BF16 = jnp.bfloat16

HQ = 32
DH = 192
M = 16
RG = 8
NG = DH // RG
NB = 4
KV_SPLIT = 1792
WQ_CUT = (0, 1792, 3840, 6144)
WO_CUT = (0, 3, 6, 9, 12, 16)
W1_LEAD = 32
W2_ROWS = 32
W2_EARLY = 20


def _kernel(x_hbm, kt_hbm, vt_hbm, wq_hbm, wo_hbm, w1_hbm, b1_hbm, w2_hbm, b2_hbm, gw_hbm,
            out_ref,
            x_v, gw_v, b1_v, b2_v, wq_v, wo_v, w1_v, w2_v, kbuf, vbuf, qh, hcol, ffn,
            small_sem, wq_sem, wo_sem, w1_sem, w2_sem, k_sem, v_sem,
            *, sk, win):
    d_model = wq_v.shape[0]
    d_ff = w1_v.shape[1]
    n_w2 = d_ff // W2_ROWS
    c0 = sk - win
    kv_cols = ((0, KV_SPLIT), (KV_SPLIT, win - KV_SPLIT))

    def copy(src, dst, sem, prio):
        pltpu.make_async_copy(src, dst, sem).start(priority=prio)

    def wait_all(buf, sem):
        pltpu.make_async_copy(buf, buf, sem).wait()

    def loop(n, body):
        def step(i, c):
            body(i)
            return c
        lax.fori_loop(0, n, step, 0)

    def rows(src_hbm, dst, sem, r, n, prio):
        r = pl.multiple_of(r, RG)
        copy(src_hbm.at[pl.ds(r, n)], dst.at[pl.ds(r, n)], sem, prio)

    def kv_piece(src_hbm, buf, sem, h, g, part, prio):
        slot = h & (NB - 1)
        col, width = kv_cols[part]
        copy(src_hbm.at[pl.ds(pl.multiple_of(h * DH + g * RG, RG), RG), pl.ds(c0 + col, width)],
             buf.at[slot, pl.ds(pl.multiple_of(g * RG, RG), RG), pl.ds(col, width)],
             sem.at[slot], prio)

    def issue_head(src_hbm, buf, sem, h):
        def body(g):
            kv_piece(src_hbm, buf, sem, h, g, 0, 0)
            kv_piece(src_hbm, buf, sem, h, g, 1, 1)
        loop(NG, body)

    def issue_parity(src_hbm, buf, sem, h0, par):
        def body(i):
            second = (i >= NG // 2).astype(jnp.int32)
            g = 2 * (i - second * (NG // 2)) + par
            kv_piece(src_hbm, buf, sem, h0 + second, g, 0, 0)
            kv_piece(src_hbm, buf, sem, h0 + second, g, 1, 1)
        loop(NG, body)

    def w2_row(j):
        return ((j & 3) * (n_w2 // 4) + (j >> 2)) * W2_ROWS

    def issue_last_v_and_w2(part):
        def body(g):
            kv_piece(vt_hbm, vbuf, v_sem, HQ - 1, g, part, 0)
            j = part * NG + g
            rows(w2_hbm, w2_v, w2_sem.at[j], w2_row(j), W2_ROWS, 1)
        loop(NG, body)

    def w1_pair(p):
        rest = (d_model // RG - W1_LEAD) // 2
        rows(w1_hbm, w1_v, w1_sem, (W1_LEAD + p) * RG, RG, 0)
        rows(w1_hbm, w1_v, w1_sem, (W1_LEAD + rest + p) * RG, RG, 1)

    def weights_pass(a):
        p0 = (3 * a) >> 1
        for n in range(15):
            j = (n - a) & 15
            r = pl.multiple_of(j * 40 + (n // 3) * RG, RG)
            ca, cb = WQ_CUT[n % 3], WQ_CUT[n % 3 + 1]
            copy(wq_hbm.at[pl.ds(r, RG), pl.ds(ca, cb - ca)],
                 wq_v.at[pl.ds(r, RG), pl.ds(ca, cb - ca)], wq_sem, 0)
            ra, rb = WO_CUT[n % 5], WO_CUT[n % 5 + 1]
            rows(wo_hbm, wo_v, wo_sem, j * 384 + (n // 5) * 128 + ra * RG, (rb - ra) * RG, 1)
            if n == 3:
                w1_pair(p0)
            if n == 11:
                @pl.when((a & 1) == 1)
                def _():
                    w1_pair(p0 + 1)

    def issue_ahead(h, which):
        h0 = (h & -2) + 2

        @pl.when(jnp.logical_and(h < HQ - 2, (h & 1) == 0))
        def _():
            issue_parity(kt_hbm, kbuf, k_sem, h0, which)

        @pl.when(jnp.logical_and(h < HQ - 3, (h & 1) == 1))
        def _():
            issue_parity(vt_hbm, vbuf, v_sem, h0, which)

        if which == 0:
            @pl.when(h == HQ - 3)
            def _():
                issue_head(vt_hbm, vbuf, v_sem, HQ - 2)
        else:
            @pl.when(h == HQ - 3)
            def _():
                issue_last_v_and_w2(0)

            @pl.when(h == HQ - 2)
            def _():
                issue_last_v_and_w2(1)

    loop(W1_LEAD, lambda i: rows(w1_hbm, w1_v, w1_sem,
                                 ((i & 1) * (W1_LEAD // 2) + (i >> 1)) * RG, RG, 1))
    loop(16, weights_pass)
    small = [(x_hbm, x_v), (gw_hbm, gw_v), (b1_hbm, b1_v), (b2_hbm, b2_v)]
    for i, (s, d) in enumerate(small):
        copy(s, d, small_sem.at[i], 0)
    issue_parity(kt_hbm, kbuf, k_sem, 0, 0)
    issue_parity(kt_hbm, kbuf, k_sem, 0, 1)
    for i, (s, d) in enumerate(small):
        pltpu.make_async_copy(s, d, small_sem.at[i]).wait()

    x = x_v[0]
    xm = jnp.broadcast_to(x, (M, d_model))

    def q_part(h0, h1):
        q = jnp.dot(xm, wq_v[:, h0 * DH:h1 * DH], preferred_element_type=F32).astype(BF16)
        for h in range(h0, h1):
            qh[h] = q[:, (h - h0) * DH:(h - h0 + 1) * DH]

    wait_all(wq_v, wq_sem)
    q_part(0, HQ // 2)
    issue_parity(vt_hbm, vbuf, v_sem, 0, 0)
    q_part(HQ // 2, HQ)
    issue_parity(vt_hbm, vbuf, v_sem, 0, 1)

    wait_all(w1_v, w1_sem)
    gate = jax.nn.sigmoid(jnp.sum(x.astype(F32) * gw_v[...].astype(F32).reshape(1, d_model),
                                  axis=1, keepdims=True))
    hid = jnp.dot(xm, w1_v[...], preferred_element_type=F32)[0:1]
    hid = jax.nn.gelu(hid + b1_v[...].astype(F32).reshape(1, d_ff), approximate=True)
    hid = hid.astype(BF16).astype(F32) * (1.0 - gate)
    for t in range(d_ff // 128):
        hcol[t * 128:(t + 1) * 128, :] = jnp.broadcast_to(hid[:, t * 128:(t + 1) * 128], (128, 128)).T
    row0 = lax.broadcasted_iota(jnp.int32, (8, d_model), 0) == 0
    ffn[...] = jnp.where(row0, (1.0 - gate) * b2_v[...].astype(F32).reshape(1, d_model), 0.0)
    wait_all(wo_v, wo_sem)

    def consume_w2(lo, hi, acc):
        def body(j, acc):
            r = pl.multiple_of(w2_row(j), W2_ROWS)
            wait_all(w2_v.at[pl.ds(r, W2_ROWS)], w2_sem.at[j])
            hc = hcol[pl.ds(r, W2_ROWS), :]
            t = w2_v[pl.ds(r, W2_ROWS), :].astype(F32) * jnp.concatenate([hc] * (d_model // 128), axis=1)
            for k in range(W2_ROWS // 8):
                acc = acc + t[k * 8:(k + 1) * 8]
            return acc
        return lax.fori_loop(lo, hi, body, acc)

    scale = DH ** -0.5

    def head(h, acc):
        slot = h & (NB - 1)
        issue_ahead(h, 0)
        wait_all(kbuf.at[slot], k_sem.at[slot])
        s = jnp.dot(qh[h], kbuf[slot], preferred_element_type=F32)[0:8] * scale
        m = jnp.max(s, axis=1, keepdims=True)
        p = jnp.exp(s - m)
        inv_l = 1.0 / jnp.sum(p, axis=1, keepdims=True)
        pb = p.astype(BF16)
        issue_ahead(h, 1)

        @pl.when(h == HQ - 1)
        def _():
            ffn[...] = consume_w2(0, W2_EARLY, ffn[...])

        wait_all(vbuf.at[slot], v_sem.at[slot])
        o = lax.dot_general(pb, vbuf[slot], (((1,), (1,)), ((), ())), preferred_element_type=F32)
        o = (o * inv_l).astype(BF16)
        r = pl.multiple_of(h * DH, 16)
        return acc + jnp.dot(o, wo_v[pl.ds(r, DH), :], preferred_element_type=F32)

    attn = lax.fori_loop(0, HQ, head, jnp.zeros((8, d_model), F32))

    tot = consume_w2(W2_EARLY, n_w2, ffn[...] + jnp.where(row0, gate * attn, 0.0))
    out_ref[0] = jnp.sum(tot, axis=0, keepdims=True).astype(out_ref.dtype)


@jax.jit
def pallas_gated_mix__sliding_block_cached__dense_activation_gelu__decode_kernel(
    A_x: jax.Array,
    A_k_cache: jax.Array,
    A_v_cache: jax.Array,
    A_wq: jax.Array,
    A_wo: jax.Array,
    B_x: jax.Array,
    B_w1: jax.Array,
    B_b1: jax.Array,
    B_w2: jax.Array,
    B_b2: jax.Array,
    gate_w: jax.Array,
):
    del B_x
    b, sq, d_model = A_x.shape
    _, hkv, sk, dh = A_k_cache.shape
    d_ff = B_w1.shape[1]
    win = min(4096, max(256, sk // 4))
    assert (b, sq, d_model, d_ff, hkv, dh, win) == (1, 1, 640, 1536, HQ, DH, 4096)
    kt = jnp.swapaxes(A_k_cache, 2, 3).reshape(HQ * DH, sk)
    vt = jnp.swapaxes(A_v_cache, 2, 3).reshape(HQ * DH, sk)

    any_spec = pl.BlockSpec(memory_space=pl.ANY)
    dma = pltpu.SemaphoreType.DMA
    return pl.pallas_call(
        functools.partial(_kernel, sk=sk, win=win),
        out_shape=jax.ShapeDtypeStruct((b, sq, d_model), A_x.dtype),
        in_specs=[any_spec] * 10,
        out_specs=pl.BlockSpec(memory_space=pltpu.VMEM),
        scratch_shapes=[
            pltpu.VMEM(A_x.shape, BF16),
            pltpu.VMEM(gate_w.shape, BF16),
            pltpu.VMEM(B_b1.shape, BF16),
            pltpu.VMEM(B_b2.shape, BF16),
            pltpu.VMEM(A_wq.shape, BF16),
            pltpu.VMEM(A_wo.shape, BF16),
            pltpu.VMEM(B_w1.shape, BF16),
            pltpu.VMEM(B_w2.shape, BF16),
            pltpu.VMEM((NB, DH, win), BF16),
            pltpu.VMEM((NB, DH, win), BF16),
            pltpu.VMEM((HQ, M, DH), BF16),
            pltpu.VMEM((d_ff, 128), F32),
            pltpu.VMEM((8, d_model), F32),
            dma((4,)), dma, dma, dma, dma((d_ff // W2_ROWS,)), dma((NB,)), dma((NB,)),
        ],
        compiler_params=pltpu.CompilerParams(
            vmem_limit_bytes=64 * 1024 * 1024,
            disable_bounds_checks=True,
            disable_semaphore_checks=True,
        ),
    )(A_x, kt, vt, A_wq, A_wo, B_w1, B_b1, B_w2, B_b2, gate_w)
```

```python
import functools

import jax
import jax.numpy as jnp
from jax import lax
import jax.experimental.pallas as pl
import jax.experimental.pallas.tpu as pltpu

F32 = jnp.float32
BF16 = jnp.bfloat16

HQ = 32
DH = 192
M = 16
RG = 8
LOG_GRP = 3
GRP = 1 << LOG_GRP
NB = 2 * GRP
BURST = DH // RG // 2
KV_SPLIT = 1792
WQ_CUT = (0, 1792, 3840, 6144)
WO_CUT = (0, 3, 6, 9, 12, 16)
W1_LEAD = 32
W2_ROWS = 32
W2_EARLY = 22
LAG = 8
LAG_LAST = 6
FIRST = 6


def _kernel(x_hbm, kt_hbm, vt_hbm, wq_hbm, wo_hbm, w1_hbm, b1_hbm, w2_hbm, b2_hbm, gw_hbm,
            out_ref,
            kbuf, vbuf, wq_v, wo_v, w1_v, w2_v, hcol, qh, ffn, xm_v, b1_f, x_v, gw_v, b1_v, b2_v,
            small_sem, wq_sem, wo_sem, w1_sem, w2_sem, k_sem, v_sem,
            *, sk, win):
    d_model = wq_v.shape[0]
    d_ff = w1_v.shape[1]
    n_w2 = d_ff // W2_ROWS
    c0 = sk - win
    kv_cols = ((0, KV_SPLIT), (KV_SPLIT, win - KV_SPLIT))

    def copy(src, dst, sem, prio):
        pltpu.make_async_copy(src, dst, sem).start(priority=prio)

    def wait_all(buf, sem):
        pltpu.make_async_copy(buf, buf, sem).wait()

    def loop(lo, hi, body):
        def step(i, c):
            body(i)
            return c
        lax.fori_loop(lo, hi, step, 0)

    def rows(src_hbm, dst, sem, r, n, prio):
        r = pl.multiple_of(r, RG)
        copy(src_hbm.at[pl.ds(r, n)], dst.at[pl.ds(r, n)], sem, prio)

    def kv_piece(src_hbm, buf, sem, h, r, part, prio):
        slot = h & (NB - 1)
        col, width = kv_cols[part]
        copy(src_hbm.at[pl.ds(pl.multiple_of(h * DH + r, RG), RG), pl.ds(c0 + col, width)],
             buf.at[slot, pl.ds(pl.multiple_of(r, RG), RG), pl.ds(col, width)],
             sem.at[slot], prio)

    def kv_burst(src_hbm, buf, sem, h, r0, step):
        def body(i):
            kv_piece(src_hbm, buf, sem, h, r0 + i * step, 0, 0)
            kv_piece(src_hbm, buf, sem, h, r0 + i * step, 1, 1)
        loop(0, BURST, body)

    def w2_row(j):
        return ((j & 3) * (n_w2 // 4) + (j >> 2)) * W2_ROWS

    def last_burst(part, g0):
        def body(g):
            kv_piece(vt_hbm, vbuf, v_sem, HQ - 1, g * RG, part, 0)
            j = part * 2 * BURST + g
            rows(w2_hbm, w2_v, w2_sem.at[j], w2_row(j), W2_ROWS, 1)
        loop(g0, g0 + BURST, body)

    tail0 = 4 * HQ - 2 * GRP
    last0 = 4 * HQ - 2
    n_bursts = last0 + 4

    def issue_burst(b):
        h = ((b >> (LOG_GRP + 2)) << LOG_GRP) + (b & (GRP - 1))
        r0 = ((b >> LOG_GRP) & 1) * RG
        is_v = ((b >> (LOG_GRP + 1)) & 1) == 1
        in_tail = b >= tail0

        @pl.when(jnp.logical_and(jnp.logical_not(is_v), b < last0))
        def _():
            kv_burst(kt_hbm, kbuf, k_sem, h, r0, 2 * RG)

        @pl.when(jnp.logical_and(is_v, b < last0))
        def _():
            kv_burst(vt_hbm, vbuf, v_sem,
                     jnp.where(in_tail, (b >> 1) - HQ, h),
                     jnp.where(in_tail, (b & 1) * (DH // 2), r0),
                     jnp.where(in_tail, RG, 2 * RG))

        for part in range(2):
            @pl.when((b >> 1) == last0 // 2 + part)
            def _():
                last_burst(part, (b & 1) * BURST)

    def bursts_before_v(h):
        regular = ((h >> LOG_GRP) << (LOG_GRP + 2)) + 3 * GRP + LAG + 2 * (h & (GRP - 1))
        return jnp.where(h < HQ - GRP, regular, jnp.minimum(2 * (HQ + h) + LAG_LAST, n_bursts))

    def w1_pair(p):
        rest = (d_model // RG - W1_LEAD) // 2
        rows(w1_hbm, w1_v, w1_sem, (W1_LEAD + p) * RG, RG, 0)
        rows(w1_hbm, w1_v, w1_sem, (W1_LEAD + rest + p) * RG, RG, 1)

    def weights_pass(a):
        p0 = (3 * a) >> 1
        for n in range(15):
            j = (n - a) & 15
            r = pl.multiple_of(j * 40 + (n // 3) * RG, RG)
            ca, cb = WQ_CUT[n % 3], WQ_CUT[n % 3 + 1]
            copy(wq_hbm.at[pl.ds(r, RG), pl.ds(ca, cb - ca)],
                 wq_v.at[pl.ds(r, RG), pl.ds(ca, cb - ca)], wq_sem, 0)
            ra, rb = WO_CUT[n % 5], WO_CUT[n % 5 + 1]
            rows(wo_hbm, wo_v, wo_sem, j * 384 + (n // 5) * 128 + ra * RG, (rb - ra) * RG, 1)
            if n == 3:
                w1_pair(p0)
            if n == 11:
                @pl.when((a & 1) == 1)
                def _():
                    w1_pair(p0 + 1)

    loop(0, W1_LEAD, lambda i: rows(w1_hbm, w1_v, w1_sem,
                                    ((i & 1) * (W1_LEAD // 2) + (i >> 1)) * RG, RG, 1))
    loop(0, 16, weights_pass)
    small = [(x_hbm, x_v), (gw_hbm, gw_v), (b1_hbm, b1_v), (b2_hbm, b2_v)]
    for i, (s, d) in enumerate(small):
        copy(s, d, small_sem.at[i], 0)
    loop(0, FIRST, lambda h: kv_burst(kt_hbm, kbuf, k_sem, h, 0, 2 * RG))
    for i, (s, d) in enumerate(small):
        pltpu.make_async_copy(s, d, small_sem.at[i]).wait()

    x = x_v[0]
    xm_v[...] = jnp.broadcast_to(x, (M, d_model))
    b1_f[...] = b1_v[...].astype(F32).reshape(1, d_ff)
    gate = jax.nn.sigmoid(jnp.sum(x.astype(F32) * gw_v[...].astype(F32).reshape(1, d_model),
                                  axis=1, keepdims=True))
    row0 = lax.broadcasted_iota(jnp.int32, (8, d_model), 0) == 0
    ffn[...] = jnp.where(row0, (1.0 - gate) * b2_v[...].astype(F32).reshape(1, d_model), 0.0)
    wait_all(wq_v, wq_sem)
    wait_all(w1_v, w1_sem)
    wait_all(wo_v, wo_sem)

    def q_pair(j):
        c = pl.multiple_of(j * (2 * DH), 128)
        q = jnp.dot(xm_v[...], wq_v[:, pl.ds(c, 2 * DH)], preferred_element_type=F32).astype(BF16)
        qh[2 * j] = q[:, :DH]
        qh[2 * j + 1] = q[:, DH:]

    def hidden_tile(t):
        c = pl.multiple_of(t * 128, 128)
        hid = jnp.dot(xm_v[...], w1_v[:, pl.ds(c, 128)], preferred_element_type=F32)[0:1]
        hid = jax.nn.gelu(hid + b1_f[:, pl.ds(c, 128)], approximate=True)
        hid = hid.astype(BF16).astype(F32) * (1.0 - gate)
        hcol[pl.ds(c, 128), :] = jnp.broadcast_to(hid, (128, 128)).T

    def consume_w2(lo, hi, acc):
        def body(j, acc):
            r = pl.multiple_of(w2_row(j), W2_ROWS)
            wait_all(w2_v.at[pl.ds(r, W2_ROWS)], w2_sem.at[j])
            hc = hcol[pl.ds(r, W2_ROWS), :]
            t = w2_v[pl.ds(r, W2_ROWS), :].astype(F32) * jnp.concatenate([hc] * (d_model // 128), axis=1)
            for k in range(W2_ROWS // 8):
                acc = acc + t[k * 8:(k + 1) * 8]
            return acc
        return lax.fori_loop(lo, hi, body, acc, unroll=2)

    scale = DH ** -0.5

    def head(h, carry):
        done, acc = carry
        slot = h & (NB - 1)
        upto = bursts_before_v(h)
        mid = jnp.maximum(upto - 1, done)
        loop(done, mid, issue_burst)

        @pl.when(h < HQ // 2)
        def _():
            q_pair(h)

        @pl.when(jnp.logical_and(h >= HQ // 2, h < HQ // 2 + d_ff // 128))
        def _():
            hidden_tile(h - HQ // 2)

        wait_all(kbuf.at[slot], k_sem.at[slot])
        s = jnp.dot(qh[h], kbuf[slot], preferred_element_type=F32)[0:8] * scale
        m = jnp.max(s, axis=1, keepdims=True)
        p = jnp.exp(s - m)
        inv_l = 1.0 / jnp.sum(p, axis=1, keepdims=True)
        pb = p.astype(BF16)
        loop(mid, upto, issue_burst)

        @pl.when(h == HQ - 1)
        def _():
            ffn[...] = consume_w2(0, W2_EARLY, ffn[...])

        wait_all(vbuf.at[slot], v_sem.at[slot])
        o = lax.dot_general(pb, vbuf[slot], (((1,), (1,)), ((), ())), preferred_element_type=F32)
        o = (o * inv_l).astype(BF16)
        r = pl.multiple_of(h * DH, 16)
        return upto, acc + jnp.dot(o, wo_v[pl.ds(r, DH), :], preferred_element_type=F32)

    _, attn = lax.fori_loop(0, HQ, head, (jnp.int32(FIRST), jnp.zeros((8, d_model), F32)))

    tot = consume_w2(W2_EARLY, n_w2, ffn[...] + jnp.where(row0, gate * attn, 0.0))
    out_ref[0] = jnp.sum(tot, axis=0, keepdims=True).astype(out_ref.dtype)


@jax.jit
def pallas_gated_mix__sliding_block_cached__dense_activation_gelu__decode_kernel(
    A_x: jax.Array,
    A_k_cache: jax.Array,
    A_v_cache: jax.Array,
    A_wq: jax.Array,
    A_wo: jax.Array,
    B_x: jax.Array,
    B_w1: jax.Array,
    B_b1: jax.Array,
    B_w2: jax.Array,
    B_b2: jax.Array,
    gate_w: jax.Array,
):
    del B_x
    b, sq, d_model = A_x.shape
    _, hkv, sk, dh = A_k_cache.shape
    d_ff = B_w1.shape[1]
    win = min(4096, max(256, sk // 4))
    assert (b, sq, d_model, d_ff, hkv, dh, win) == (1, 1, 640, 1536, HQ, DH, 4096)
    kt = jnp.swapaxes(A_k_cache, 2, 3).reshape(HQ * DH, sk)
    vt = jnp.swapaxes(A_v_cache, 2, 3).reshape(HQ * DH, sk)

    any_spec = pl.BlockSpec(memory_space=pl.ANY)
    dma = pltpu.SemaphoreType.DMA
    return pl.pallas_call(
        functools.partial(_kernel, sk=sk, win=win),
        out_shape=jax.ShapeDtypeStruct((b, sq, d_model), A_x.dtype),
        in_specs=[any_spec] * 10,
        out_specs=pl.BlockSpec(memory_space=pltpu.VMEM),
        scratch_shapes=[
            pltpu.VMEM((NB, DH, win), BF16),
            pltpu.VMEM((NB, DH, win), BF16),
            pltpu.VMEM(A_wq.shape, BF16),
            pltpu.VMEM(A_wo.shape, BF16),
            pltpu.VMEM(B_w1.shape, BF16),
            pltpu.VMEM(B_w2.shape, BF16),
            pltpu.VMEM((d_ff, 128), F32),
            pltpu.VMEM((HQ, M, DH), BF16),
            pltpu.VMEM((8, d_model), F32),
            pltpu.VMEM((M, d_model), BF16),
            pltpu.VMEM((1, d_ff), F32),
            pltpu.VMEM(A_x.shape, BF16),
            pltpu.VMEM(gate_w.shape, BF16),
            pltpu.VMEM(B_b1.shape, BF16),
            pltpu.VMEM(B_b2.shape, BF16),
            dma((4,)), dma, dma, dma, dma((d_ff // W2_ROWS,)), dma((NB,)), dma((NB,)),
        ],
        compiler_params=pltpu.CompilerParams(
            vmem_limit_bytes=100 * 1024 * 1024,
            disable_bounds_checks=True,
            disable_semaphore_checks=True,
        ),
    )(A_x, kt, vt, A_wq, A_wo, B_w1, B_b1, B_w2, B_b2, gate_w)
```

```python
import functools

import jax
import jax.numpy as jnp
from jax import lax
import jax.experimental.pallas as pl
import jax.experimental.pallas.tpu as pltpu

F32 = jnp.float32
BF16 = jnp.bfloat16

HQ = 32
DH = 192
M = 16
RG = 8
LOG_GRP = 3
GRP = 1 << LOG_GRP
NB = 2 * GRP
BURST = DH // RG // 2
KV_SPLIT = 1792
WQ_CUT = (0, 1792, 3840, 6144)
WO_CUT = (0, 3, 6, 9, 12, 16)
W1_LEAD = 32
W2_ROWS = 32
W2_EARLY = 22
LAG = 8
LAG_LAST = 6
FIRST = 6


def _kernel(x_hbm, kt_hbm, vt_hbm, wq_hbm, wo_hbm, w1_hbm, b1_hbm, w2_hbm, b2_hbm, gw_hbm,
            out_ref,
            kbuf, vbuf, wq_v, wo_v, w1_v, w2_v, hcol, qh, ffn, xm_v, b1_f, x_v, gw_v, b1_v, b2_v,
            small_sem, wq_sem, wo_sem, w1_sem, w2_sem, k_sem, v_sem,
            *, sk, win):
    d_model = wq_v.shape[0]
    d_ff = w1_v.shape[1]
    n_w2 = d_ff // W2_ROWS
    c0 = sk - win
    kv_cols = ((0, KV_SPLIT), (KV_SPLIT, win - KV_SPLIT))

    def copy(src, dst, sem, prio):
        pltpu.make_async_copy(src, dst, sem).start(priority=prio)

    def wait_all(buf, sem):
        pltpu.make_async_copy(buf, buf, sem).wait()

    def loop(lo, hi, body):
        def step(i, c):
            body(i)
            return c
        lax.fori_loop(lo, hi, step, 0)

    def rows(src_hbm, dst, sem, r, n, prio):
        r = pl.multiple_of(r, RG)
        copy(src_hbm.at[pl.ds(r, n)], dst.at[pl.ds(r, n)], sem, prio)

    def kv_piece(src_hbm, buf, sem, h, r, part, prio):
        slot = h & (NB - 1)
        col, width = kv_cols[part]
        copy(src_hbm.at[pl.ds(pl.multiple_of(h * DH + r, RG), RG), pl.ds(c0 + col, width)],
             buf.at[slot, pl.ds(pl.multiple_of(r, RG), RG), pl.ds(col, width)],
             sem.at[slot], prio)

    def kv_burst(src_hbm, buf, sem, h, r0, step):
        def body(i):
            kv_piece(src_hbm, buf, sem, h, r0 + i * step, 0, 0)
            kv_piece(src_hbm, buf, sem, h, r0 + i * step, 1, 1)
        loop(0, BURST, body)

    def w2_row(j):
        return ((j & 3) * (n_w2 // 4) + (j >> 2)) * W2_ROWS

    def last_burst(part, g0):
        def body(g):
            kv_piece(vt_hbm, vbuf, v_sem, HQ - 1, g * RG, part, 0)
            j = part * 2 * BURST + g
            rows(w2_hbm, w2_v, w2_sem.at[j], w2_row(j), W2_ROWS, 1)
        loop(g0, g0 + BURST, body)

    tail0 = 4 * HQ - 2 * GRP
    last0 = 4 * HQ - 2
    n_bursts = last0 + 4

    def issue_burst(b):
        h = ((b >> (LOG_GRP + 2)) << LOG_GRP) + (b & (GRP - 1))
        r0 = ((b >> LOG_GRP) & 1) * RG
        is_v = ((b >> (LOG_GRP + 1)) & 1) == 1
        in_tail = b >= tail0

        @pl.when(jnp.logical_and(jnp.logical_not(is_v), b < last0))
        def _():
            kv_burst(kt_hbm, kbuf, k_sem, h, r0, 2 * RG)

        @pl.when(jnp.logical_and(is_v, b < last0))
        def _():
            kv_burst(vt_hbm, vbuf, v_sem,
                     jnp.where(in_tail, (b >> 1) - HQ, h),
                     jnp.where(in_tail, (b & 1) * (DH // 2), r0),
                     jnp.where(in_tail, RG, 2 * RG))

        for part in range(2):
            @pl.when((b >> 1) == last0 // 2 + part)
            def _():
                last_burst(part, (b & 1) * BURST)

    def bursts_before_v(h):
        regular = ((h >> LOG_GRP) << (LOG_GRP + 2)) + 3 * GRP + LAG + 2 * (h & (GRP - 1))
        return jnp.where(h < HQ - GRP, regular, jnp.minimum(2 * (HQ + h) + LAG_LAST, n_bursts))

    def w1_pair(p):
        rest = (d_model // RG - W1_LEAD) // 2
        rows(w1_hbm, w1_v, w1_sem, (W1_LEAD + p) * RG, RG, 0)
        rows(w1_hbm, w1_v, w1_sem, (W1_LEAD + rest + p) * RG, RG, 1)

    def weights_pass(a):
        p0 = (3 * a) >> 1
        for m in range(15):
            n = (2 * m) % 15
            j = (n - a) & 15
            r = pl.multiple_of(j * 40 + (n // 3) * RG, RG)
            ca, cb = WQ_CUT[n % 3], WQ_CUT[n % 3 + 1]
            copy(wq_hbm.at[pl.ds(r, RG), pl.ds(ca, cb - ca)],
                 wq_v.at[pl.ds(r, RG), pl.ds(ca, cb - ca)], wq_sem, 0)
            ra, rb = WO_CUT[n % 5], WO_CUT[n % 5 + 1]
            rows(wo_hbm, wo_v, wo_sem, j * 384 + (n // 5) * 128 + ra * RG, (rb - ra) * RG, 1)
            if m == 3:
                w1_pair(p0)
            if m == 11:
                @pl.when((a & 1) == 1)
                def _():
                    w1_pair(p0 + 1)

    loop(0, W1_LEAD, lambda i: rows(w1_hbm, w1_v, w1_sem,
                                    ((i & 1) * (W1_LEAD // 2) + (i >> 1)) * RG, RG, 1))
    loop(0, 16, weights_pass)
    small = [(x_hbm, x_v), (gw_hbm, gw_v), (b1_hbm, b1_v), (b2_hbm, b2_v)]
    for i, (s, d) in enumerate(small):
        copy(s, d, small_sem.at[i], 0)
    loop(0, FIRST, lambda h: kv_burst(kt_hbm, kbuf, k_sem, h, 0, 2 * RG))
    for i, (s, d) in enumerate(small):
        pltpu.make_async_copy(s, d, small_sem.at[i]).wait()

    x = x_v[0]
    xm_v[...] = jnp.broadcast_to(x, (M, d_model))
    b1_f[...] = b1_v[...].astype(F32).reshape(1, d_ff)
    gate = jax.nn.sigmoid(jnp.sum(x.astype(F32) * gw_v[...].astype(F32).reshape(1, d_model),
                                  axis=1, keepdims=True))
    row0 = lax.broadcasted_iota(jnp.int32, (8, d_model), 0) == 0
    ffn[...] = jnp.where(row0, (1.0 - gate) * b2_v[...].astype(F32).reshape(1, d_model), 0.0)
    wait_all(wq_v, wq_sem)
    wait_all(w1_v, w1_sem)
    wait_all(wo_v, wo_sem)

    def q_pair(j):
        c = pl.multiple_of(j * (2 * DH), 128)
        q = jnp.dot(xm_v[...], wq_v[:, pl.ds(c, 2 * DH)], preferred_element_type=F32).astype(BF16)
        qh[2 * j] = q[:, :DH]
        qh[2 * j + 1] = q[:, DH:]

    def hidden_tile(t):
        c = pl.multiple_of(t * 128, 128)
        hid = jnp.dot(xm_v[...], w1_v[:, pl.ds(c, 128)], preferred_element_type=F32)[0:1]
        hid = jax.nn.gelu(hid + b1_f[:, pl.ds(c, 128)], approximate=True)
        hid = hid.astype(BF16).astype(F32) * (1.0 - gate)
        hcol[pl.ds(c, 128), :] = jnp.broadcast_to(hid, (128, 128)).T

    def consume_w2(lo, hi, acc):
        def body(j, acc):
            r = pl.multiple_of(w2_row(j), W2_ROWS)
            wait_all(w2_v.at[pl.ds(r, W2_ROWS)], w2_sem.at[j])
            hc = hcol[pl.ds(r, W2_ROWS), :]
            t = w2_v[pl.ds(r, W2_ROWS), :].astype(F32) * jnp.concatenate([hc] * (d_model // 128), axis=1)
            for k in range(W2_ROWS // 8):
                acc = acc + t[k * 8:(k + 1) * 8]
            return acc
        return lax.fori_loop(lo, hi, body, acc, unroll=2)

    scale = DH ** -0.5

    def head(h, carry):
        done, acc = carry
        slot = h & (NB - 1)
        upto = bursts_before_v(h)
        mid = jnp.maximum(upto - 1, done)
        loop(done, mid, issue_burst)

        @pl.when(h < HQ // 2)
        def _():
            q_pair(h)

        @pl.when(jnp.logical_and(h >= HQ // 2, h < HQ // 2 + d_ff // 128))
        def _():
            hidden_tile(h - HQ // 2)

        wait_all(kbuf.at[slot], k_sem.at[slot])
        s = jnp.dot(qh[h], kbuf[slot], preferred_element_type=F32)[0:8] * scale
        m = jnp.max(s, axis=1, keepdims=True)
        p = jnp.exp(s - m)
        inv_l = 1.0 / jnp.sum(p, axis=1, keepdims=True)
        pb = p.astype(BF16)
        loop(mid, upto, issue_burst)

        @pl.when(h == HQ - 1)
        def _():
            ffn[...] = consume_w2(0, W2_EARLY, ffn[...])

        wait_all(vbuf.at[slot], v_sem.at[slot])
        o = lax.dot_general(pb, vbuf[slot], (((1,), (1,)), ((), ())), preferred_element_type=F32)
        o = (o * inv_l).astype(BF16)
        r = pl.multiple_of(h * DH, 16)
        return upto, acc + jnp.dot(o, wo_v[pl.ds(r, DH), :], preferred_element_type=F32)

    _, attn = lax.fori_loop(0, HQ, head, (jnp.int32(FIRST), jnp.zeros((8, d_model), F32)))

    tot = consume_w2(W2_EARLY, n_w2, ffn[...] + jnp.where(row0, gate * attn, 0.0))
    out_ref[0] = jnp.sum(tot, axis=0, keepdims=True).astype(out_ref.dtype)


def _compiler_params():
    params = dict(vmem_limit_bytes=96 * 1024 * 1024, disable_bounds_checks=True)
    try:
        return pltpu.CompilerParams(disable_semaphore_checks=True, **params)
    except TypeError:
        return pltpu.CompilerParams(**params)


@jax.jit
def pallas_gated_mix__sliding_block_cached__dense_activation_gelu__decode_kernel(
    A_x: jax.Array,
    A_k_cache: jax.Array,
    A_v_cache: jax.Array,
    A_wq: jax.Array,
    A_wo: jax.Array,
    B_x: jax.Array,
    B_w1: jax.Array,
    B_b1: jax.Array,
    B_w2: jax.Array,
    B_b2: jax.Array,
    gate_w: jax.Array,
):
    del B_x
    b, sq, d_model = A_x.shape
    _, hkv, sk, dh = A_k_cache.shape
    d_ff = B_w1.shape[1]
    win = min(4096, max(256, sk // 4))
    assert (b, sq, d_model, d_ff, hkv, dh, win) == (1, 1, 640, 1536, HQ, DH, 4096)
    kt = jnp.swapaxes(A_k_cache, 2, 3).reshape(HQ * DH, sk)
    vt = jnp.swapaxes(A_v_cache, 2, 3).reshape(HQ * DH, sk)

    any_spec = pl.BlockSpec(memory_space=pl.ANY)
    dma = pltpu.SemaphoreType.DMA
    return pl.pallas_call(
        functools.partial(_kernel, sk=sk, win=win),
        out_shape=jax.ShapeDtypeStruct((b, sq, d_model), A_x.dtype),
        in_specs=[any_spec] * 10,
        out_specs=pl.BlockSpec(memory_space=pltpu.VMEM),
        scratch_shapes=[
            pltpu.VMEM((NB, DH, win), BF16),
            pltpu.VMEM((NB, DH, win), BF16),
            pltpu.VMEM(A_wq.shape, BF16),
            pltpu.VMEM(A_wo.shape, BF16),
            pltpu.VMEM(B_w1.shape, BF16),
            pltpu.VMEM(B_w2.shape, BF16),
            pltpu.VMEM((d_ff, 128), F32),
            pltpu.VMEM((HQ, M, DH), BF16),
            pltpu.VMEM((8, d_model), F32),
            pltpu.VMEM((M, d_model), BF16),
            pltpu.VMEM((1, d_ff), F32),
            pltpu.VMEM(A_x.shape, BF16),
            pltpu.VMEM(gate_w.shape, BF16),
            pltpu.VMEM(B_b1.shape, BF16),
            pltpu.VMEM(B_b2.shape, BF16),
            dma((4,)), dma, dma, dma, dma((d_ff // W2_ROWS,)), dma((NB,)), dma((NB,)),
        ],
        compiler_params=_compiler_params(),
    )(A_x, kt, vt, A_wq, A_wo, B_w1, B_b1, B_w2, B_b2, gate_w)
```

```python
import functools

import jax
import jax.numpy as jnp
from jax import lax
import jax.experimental.pallas as pl
import jax.experimental.pallas.tpu as pltpu

F32 = jnp.float32
BF16 = jnp.bfloat16

HQ = 32
DH = 192
M = 16
RG = 8
BURST = DH // RG // 2
TILE_OFF = 2
KV_SPLIT = (16 - TILE_OFF) * 128
W1_LEAD = 32
W2_ROWS = 32
W2_EARLY = 22
FIRST = 6
LAG = 6


def _kernel(x_hbm, kt_hbm, vt_hbm, wq_hbm, wo_hbm, w1_hbm, b1_hbm, w2_hbm, b2_hbm, gw_hbm,
            out_ref,
            kv, p_all, wq_v, wo_v, w1_v, w2_v, hcol, qh, ffn, xm_v, b1_f, x_v, gw_v, b1_v, b2_v,
            w_sem, w2_sem, kv_sem,
            *, sk, win):
    d_model = wq_v.shape[0]
    d_ff = w1_v.shape[1]
    n_w2 = d_ff // W2_ROWS
    c0 = sk - win
    kv_cols = ((0, KV_SPLIT), (KV_SPLIT, win - KV_SPLIT))
    wq_sem, wo_sem, w1_sem = w_sem.at[4], w_sem.at[5], w_sem.at[6]

    def copy(src, dst, sem, prio):
        pltpu.make_async_copy(src, dst, sem).start(priority=prio)

    def wait_all(buf, sem):
        pltpu.make_async_copy(buf, buf, sem).wait()

    def loop(lo, hi, body):
        def step(i, c):
            body(i)
            return c
        lax.fori_loop(lo, hi, step, 0)

    def rows(src_hbm, dst, sem, r, n, prio):
        r = pl.multiple_of(r, RG)
        copy(src_hbm.at[pl.ds(r, n)], dst.at[pl.ds(r, n)], sem, prio)

    def kv_piece(src_hbm, h, r, part, prio):
        col, width = kv_cols[part]
        copy(src_hbm.at[pl.ds(pl.multiple_of(h * DH + r, RG), RG), pl.ds(c0 + col, width)],
             kv.at[h, pl.ds(pl.multiple_of(r, RG), RG), pl.ds(col, width)],
             kv_sem.at[h], prio)

    def kv_burst(src_hbm, h, odd):
        def body(i):
            kv_piece(src_hbm, h, (2 * i + odd) * RG, 1, 0)
            kv_piece(src_hbm, h, (2 * i + odd) * RG, 0, 1)
        loop(0, BURST, body)

    def w2_row(j):
        return ((j & 3) * (n_w2 // 4) + (j >> 2)) * W2_ROWS

    def last_burst(part, g0):
        def body(g):
            kv_piece(vt_hbm, HQ - 1, g * RG, part, 0)
            j = part * 2 * BURST + g
            rows(w2_hbm, w2_v, w2_sem.at[j], w2_row(j), W2_ROWS, 1)
        loop(g0, g0 + BURST, body)

    def w1_pair(p):
        rest = (d_model // RG - W1_LEAD) // 2
        rows(w1_hbm, w1_v, w1_sem, (W1_LEAD + p) * RG, RG, 0)
        rows(w1_hbm, w1_v, w1_sem, (W1_LEAD + rest + p) * RG, RG, 1)

    def block(src_hbm, dst, sem, j, n, prio):
        tpr = dst.shape[1] // 128
        per = 240 // tpr * RG
        lo, hi = 16 * n - TILE_OFF, 16 * n + 16 - TILE_OFF
        while lo < hi:
            g, c = divmod(lo, tpr)
            if c == 0 and hi - lo >= tpr:
                cnt = (hi - lo) // tpr
                rows(src_hbm, dst, sem, j * per + g * RG, cnt * RG, prio)
                lo += cnt * tpr
            else:
                e = min(hi, (g + 1) * tpr)
                r = j * per + g * RG if g >= 0 else ((j - 1) & 15) * per + per + g * RG
                r = pl.multiple_of(r, RG)
                copy(src_hbm.at[pl.ds(r, RG), pl.ds(c * 128, (e - lo) * 128)],
                     dst.at[pl.ds(r, RG), pl.ds(c * 128, (e - lo) * 128)], sem, prio)
                lo = e

    def weights_pass(a):
        p0 = (3 * a) >> 1
        for m in range(15):
            n = (4 * m) % 15
            j = (n - a) & 15
            block(wq_hbm, wq_v, wq_sem, j, n, 0)
            block(wo_hbm, wo_v, wo_sem, j, n, 1)
            if m == 3:
                w1_pair(p0)
            if m == 11:
                @pl.when((a & 1) == 1)
                def _():
                    w1_pair(p0 + 1)

    for i in range(W1_LEAD):
        r = ((i & 1) * (W1_LEAD // 2) + (i >> 1)) * RG
        copy(w1_hbm.at[pl.ds(r, RG)], w1_v.at[pl.ds(r, RG)], w1_sem, 0 if i % 16 == 1 else 1)
    loop(0, 16, weights_pass)
    small = [(x_hbm, x_v), (gw_hbm, gw_v), (b1_hbm, b1_v), (b2_hbm, b2_v)]
    for i, (s, d) in enumerate(small):
        copy(s, d, w_sem.at[i], 0)
    loop(0, FIRST, lambda h: kv_burst(kt_hbm, h, 0))
    for i, (s, d) in enumerate(small):
        pltpu.make_async_copy(s, d, w_sem.at[i]).wait()

    x = x_v[0]
    xm_v[...] = jnp.broadcast_to(x, (M, d_model))
    b1_f[...] = b1_v[...].astype(F32).reshape(1, d_ff)
    gate = jax.nn.sigmoid(jnp.sum(x.astype(F32) * gw_v[...].astype(F32).reshape(1, d_model),
                                  axis=1, keepdims=True))
    row0 = lax.broadcasted_iota(jnp.int32, (8, d_model), 0) == 0
    ffn[...] = jnp.where(row0, (1.0 - gate) * b2_v[...].astype(F32).reshape(1, d_model), 0.0)
    wait_all(wq_v, wq_sem)
    wait_all(w1_v, w1_sem)
    wait_all(wo_v, wo_sem)

    def q_pair(j):
        c = pl.multiple_of(j * (2 * DH), 128)
        q = jnp.dot(xm_v[...], wq_v[:, pl.ds(c, 2 * DH)], preferred_element_type=F32).astype(BF16)
        qh[2 * j] = q[:, :DH]
        qh[2 * j + 1] = q[:, DH:]

    def hidden_tile(t):
        c = pl.multiple_of(t * 128, 128)
        hid = jnp.dot(xm_v[...], w1_v[:, pl.ds(c, 128)], preferred_element_type=F32)[0:1]
        hid = jax.nn.gelu(hid + b1_f[:, pl.ds(c, 128)], approximate=True)
        hid = hid.astype(BF16).astype(F32) * (1.0 - gate)
        hcol[pl.ds(c, 128), :] = jnp.broadcast_to(hid, (128, 128)).T

    def consume_w2(lo, hi, acc):
        def body(j, acc):
            r = pl.multiple_of(w2_row(j), W2_ROWS)
            wait_all(w2_v.at[pl.ds(r, W2_ROWS)], w2_sem.at[j])
            hc = hcol[pl.ds(r, W2_ROWS), :]
            t = w2_v[pl.ds(r, W2_ROWS), :].astype(F32) * jnp.concatenate([hc] * (d_model // 128), axis=1)
            for k in range(W2_ROWS // 8):
                acc = acc + t[k * 8:(k + 1) * 8]
            return acc
        return lax.fori_loop(lo, hi, body, acc, unroll=2)

    scale = DH ** -0.5

    def k_even(h):
        kv_burst(kt_hbm, h, 0)

        @pl.when(h < FIRST + HQ // 2)
        def _():
            q_pair(h - FIRST)

    loop(FIRST, HQ, k_even)
    loop(0, LAG, lambda h: kv_burst(kt_hbm, h, 1))

    def scores(h):
        @pl.when(h < HQ - LAG)
        def _():
            kv_burst(kt_hbm, h + LAG, 1)

        @pl.when(h >= HQ - LAG)
        def _():
            kv_burst(vt_hbm, h - (HQ - LAG), 0)

        wait_all(kv.at[h], kv_sem.at[h])
        s = jnp.dot(qh[h], kv[h], preferred_element_type=F32)[0:8] * scale
        p = jnp.exp(s - jnp.max(s, axis=1, keepdims=True))
        p_all[h] = (p * (1.0 / jnp.sum(p, axis=1, keepdims=True))).astype(BF16)

    loop(0, HQ, scores)

    def v_even(h):
        kv_burst(vt_hbm, h, 0)

        @pl.when(h < LAG + d_ff // 128)
        def _():
            hidden_tile(h - LAG)

    loop(LAG, HQ - 1, v_even)
    loop(0, LAG, lambda h: kv_burst(vt_hbm, h, 1))

    def values(h, acc):
        @pl.when(h < HQ - 1 - LAG)
        def _():
            kv_burst(vt_hbm, h + LAG, 1)

        t = h - (HQ - 1 - LAG)
        for part in range(2):
            @pl.when((t >> 1) == part)
            def _():
                last_burst(part, (t & 1) * BURST)

        @pl.when(h == HQ - 1)
        def _():
            ffn[...] = consume_w2(0, W2_EARLY, ffn[...])

        wait_all(kv.at[h], kv_sem.at[h])
        o = lax.dot_general(p_all[h], kv[h], (((1,), (1,)), ((), ())), preferred_element_type=F32)
        r = pl.multiple_of(h * DH, 16)
        return acc + jnp.dot(o.astype(BF16), wo_v[pl.ds(r, DH), :], preferred_element_type=F32)

    attn = lax.fori_loop(0, HQ, values, jnp.zeros((8, d_model), F32))

    tot = consume_w2(W2_EARLY, n_w2, ffn[...] + jnp.where(row0, gate * attn, 0.0))
    out_ref[0] = jnp.sum(tot, axis=0, keepdims=True).astype(out_ref.dtype)


def _compiler_params():
    params = dict(vmem_limit_bytes=96 * 1024 * 1024, disable_bounds_checks=True)
    try:
        return pltpu.CompilerParams(disable_semaphore_checks=True, **params)
    except TypeError:
        return pltpu.CompilerParams(**params)


@jax.jit
def pallas_gated_mix__sliding_block_cached__dense_activation_gelu__decode_kernel(
    A_x: jax.Array,
    A_k_cache: jax.Array,
    A_v_cache: jax.Array,
    A_wq: jax.Array,
    A_wo: jax.Array,
    B_x: jax.Array,
    B_w1: jax.Array,
    B_b1: jax.Array,
    B_w2: jax.Array,
    B_b2: jax.Array,
    gate_w: jax.Array,
):
    del B_x
    b, sq, d_model = A_x.shape
    _, hkv, sk, dh = A_k_cache.shape
    d_ff = B_w1.shape[1]
    win = min(4096, max(256, sk // 4))
    assert (b, sq, d_model, d_ff, hkv, dh, win) == (1, 1, 640, 1536, HQ, DH, 4096)
    kt = jnp.swapaxes(A_k_cache, 2, 3).reshape(HQ * DH, sk)
    vt = jnp.swapaxes(A_v_cache, 2, 3).reshape(HQ * DH, sk)

    any_spec = pl.BlockSpec(memory_space=pl.ANY)
    dma = pltpu.SemaphoreType.DMA
    return pl.pallas_call(
        functools.partial(_kernel, sk=sk, win=win),
        out_shape=jax.ShapeDtypeStruct((b, sq, d_model), A_x.dtype),
        in_specs=[any_spec] * 10,
        out_specs=pl.BlockSpec(memory_space=pltpu.VMEM),
        scratch_shapes=[
            pltpu.VMEM((HQ, DH, win), BF16),
            pltpu.VMEM((HQ, 8, win), BF16),
            pltpu.VMEM(A_wq.shape, BF16),
            pltpu.VMEM(A_wo.shape, BF16),
            pltpu.VMEM(B_w1.shape, BF16),
            pltpu.VMEM(B_w2.shape, BF16),
            pltpu.VMEM((d_ff, 128), F32),
            pltpu.VMEM((HQ, M, DH), BF16),
            pltpu.VMEM((8, d_model), F32),
            pltpu.VMEM((M, d_model), BF16),
            pltpu.VMEM((1, d_ff), F32),
            pltpu.VMEM(A_x.shape, BF16),
            pltpu.VMEM(gate_w.shape, BF16),
            pltpu.VMEM(B_b1.shape, BF16),
            pltpu.VMEM(B_b2.shape, BF16),
            dma((7,)), dma((d_ff // W2_ROWS,)), dma((HQ,)),
        ],
        compiler_params=_compiler_params(),
    )(A_x, kt, vt, A_wq, A_wo, B_w1, B_b1, B_w2, B_b2, gate_w)
```

```python
import functools

import jax
import jax.numpy as jnp
from jax import lax
import jax.experimental.pallas as pl
import jax.experimental.pallas.tpu as pltpu

F32 = jnp.float32
BF16 = jnp.bfloat16

HQ = 32
DH = 192
M = 16
RG = 8
BURST = DH // RG // 2
TILE_OFF = 2
KV_SPLIT = (16 - TILE_OFF) * 128
W1_LEAD = 32
W2_ROWS = 32
W2_EARLY = 22
FIRST = 6
LAG = 6


def _kernel(x_hbm, kt_hbm, vt_hbm, wq_hbm, wo_hbm, w1_hbm, b1_hbm, w2_hbm, b2_hbm, gw_hbm,
            out_ref,
            kv, p_all, wq_v, wo_v, w1_v, w2_v, hcol, qh, ffn, xm_v, b1_f, x_v, gw_v, b1_v, b2_v,
            w_sem, w2_sem, kv_sem,
            *, sk, win):
    d_model = wq_v.shape[0]
    d_ff = w1_v.shape[1]
    n_w2 = d_ff // W2_ROWS
    c0 = sk - win
    kv_cols = ((0, KV_SPLIT), (KV_SPLIT, win - KV_SPLIT))
    wq_sem, wo_sem, w1_sem = w_sem.at[4], w_sem.at[5], w_sem.at[6]

    def copy(src, dst, sem, prio):
        pltpu.make_async_copy(src, dst, sem).start(priority=prio)

    def wait_all(buf, sem):
        pltpu.make_async_copy(buf, buf, sem).wait()

    def loop(lo, hi, body):
        def step(i, c):
            body(i)
            return c
        lax.fori_loop(lo, hi, step, 0)

    def rows(src_hbm, dst, sem, r, n, prio):
        r = pl.multiple_of(r, RG)
        copy(src_hbm.at[pl.ds(r, n)], dst.at[pl.ds(r, n)], sem, prio)

    def kv_piece(src_hbm, h, r, part, prio):
        col, width = kv_cols[part]
        copy(src_hbm.at[pl.ds(pl.multiple_of(h * DH + r, RG), RG), pl.ds(c0 + col, width)],
             kv.at[h, pl.ds(pl.multiple_of(r, RG), RG), pl.ds(col, width)],
             kv_sem.at[h], prio)

    def kv_burst(src_hbm, h, odd):
        def body(i):
            kv_piece(src_hbm, h, (2 * i + odd) * RG, 1, 0)
            kv_piece(src_hbm, h, (2 * i + odd) * RG, 0, 1)
        loop(0, BURST, body)

    def w2_row(j):
        return ((j & 3) * (n_w2 // 4) + (j >> 2)) * W2_ROWS

    def last_burst(part, g0):
        def body(g):
            kv_piece(vt_hbm, HQ - 1, g * RG, part, 0)
            j = part * 2 * BURST + g
            rows(w2_hbm, w2_v, w2_sem.at[j], w2_row(j), W2_ROWS, 1)
        loop(g0, g0 + BURST, body)

    def w1_pair(p):
        rest = (d_model // RG - W1_LEAD) // 2
        rows(w1_hbm, w1_v, w1_sem, (W1_LEAD + p) * RG, RG, 0)
        rows(w1_hbm, w1_v, w1_sem, (W1_LEAD + rest + p) * RG, RG, 1)

    def block(src_hbm, dst, sem, j, n, prio):
        tpr = dst.shape[1] // 128
        per = 240 // tpr * RG
        lo, hi = 16 * n - TILE_OFF, 16 * n + 16 - TILE_OFF
        while lo < hi:
            g, c = divmod(lo, tpr)
            if c == 0 and hi - lo >= tpr:
                cnt = (hi - lo) // tpr
                rows(src_hbm, dst, sem, j * per + g * RG, cnt * RG, prio)
                lo += cnt * tpr
            else:
                e = min(hi, (g + 1) * tpr)
                r = j * per + g * RG if g >= 0 else ((j - 1) & 15) * per + per + g * RG
                r = pl.multiple_of(r, RG)
                copy(src_hbm.at[pl.ds(r, RG), pl.ds(c * 128, (e - lo) * 128)],
                     dst.at[pl.ds(r, RG), pl.ds(c * 128, (e - lo) * 128)], sem, prio)
                lo = e

    def weights_pass(a):
        p0 = (3 * a) >> 1
        for m in range(15):
            n = (4 * m) % 15
            j = (n - a) & 15
            block(wq_hbm, wq_v, wq_sem, j, n, 0)
            block(wo_hbm, wo_v, wo_sem, j, n, 1)
            if m == 3:
                w1_pair(p0)
            if m == 11:
                @pl.when((a & 1) == 1)
                def _():
                    w1_pair(p0 + 1)

    for i in range(W1_LEAD):
        r = ((i & 1) * (W1_LEAD // 2) + (i >> 1)) * RG
        copy(w1_hbm.at[pl.ds(r, RG)], w1_v.at[pl.ds(r, RG)], w1_sem, 0 if i % 16 == 1 else 1)
    loop(0, 16, weights_pass)
    small = [(x_hbm, x_v), (gw_hbm, gw_v), (b1_hbm, b1_v), (b2_hbm, b2_v)]
    for i, (s, d) in enumerate(small):
        copy(s, d, w_sem.at[i], 0)
    loop(0, FIRST, lambda h: kv_burst(kt_hbm, h, 0))
    for i, (s, d) in enumerate(small):
        pltpu.make_async_copy(s, d, w_sem.at[i]).wait()

    x = x_v[0]
    xm_v[...] = jnp.broadcast_to(x, (M, d_model))
    b1_f[...] = b1_v[...].astype(F32).reshape(1, d_ff)
    gate = jax.nn.sigmoid(jnp.sum(x.astype(F32) * gw_v[...].astype(F32).reshape(1, d_model),
                                  axis=1, keepdims=True))
    row0 = lax.broadcasted_iota(jnp.int32, (8, d_model), 0) == 0
    ffn[...] = jnp.where(row0, (1.0 - gate) * b2_v[...].astype(F32).reshape(1, d_model), 0.0)
    wait_all(wq_v, wq_sem)
    wait_all(w1_v, w1_sem)
    wait_all(wo_v, wo_sem)

    def q_pair(j):
        c = pl.multiple_of(j * (2 * DH), 128)
        q = jnp.dot(xm_v[...], wq_v[:, pl.ds(c, 2 * DH)], preferred_element_type=F32).astype(BF16)
        qh[2 * j] = q[:, :DH]
        qh[2 * j + 1] = q[:, DH:]

    def hidden_tile(t):
        c = pl.multiple_of(t * 128, 128)
        hid = jnp.dot(xm_v[...], w1_v[:, pl.ds(c, 128)], preferred_element_type=F32)[0:1]
        hid = jax.nn.gelu(hid + b1_f[:, pl.ds(c, 128)], approximate=True)
        hid = hid.astype(BF16).astype(F32) * (1.0 - gate)
        hcol[pl.ds(c, 128), :] = jnp.broadcast_to(hid, (128, 128)).T

    def consume_w2(lo, hi, acc):
        def body(j, acc):
            r = pl.multiple_of(w2_row(j), W2_ROWS)
            wait_all(w2_v.at[pl.ds(r, W2_ROWS)], w2_sem.at[j])
            hc = hcol[pl.ds(r, W2_ROWS), :]
            t = w2_v[pl.ds(r, W2_ROWS), :].astype(F32) * jnp.concatenate([hc] * (d_model // 128), axis=1)
            for k in range(W2_ROWS // 8):
                acc = acc + t[k * 8:(k + 1) * 8]
            return acc
        return lax.fori_loop(lo, hi, body, acc, unroll=2)

    scale = DH ** -0.5

    def k_even(h):
        kv_burst(kt_hbm, h, 0)

        @pl.when(h < FIRST + HQ // 2)
        def _():
            q_pair(h - FIRST)

    loop(FIRST, HQ, k_even)
    loop(0, LAG, lambda h: kv_burst(kt_hbm, h, 1))

    def scores(h):
        @pl.when(h < HQ - LAG)
        def _():
            kv_burst(kt_hbm, h + LAG, 1)

        @pl.when(h >= HQ - LAG)
        def _():
            kv_burst(vt_hbm, h - (HQ - LAG), 0)

        wait_all(kv.at[h], kv_sem.at[h])
        s = jnp.dot(qh[h], kv[h], preferred_element_type=F32)[0:8] * scale
        p = jnp.exp(s - jnp.max(s, axis=1, keepdims=True))
        p_all[h] = (p * (1.0 / jnp.sum(p, axis=1, keepdims=True))).astype(BF16)

    loop(0, HQ, scores)

    def v_even(h):
        kv_burst(vt_hbm, h, 0)

        @pl.when(h < LAG + d_ff // 128)
        def _():
            hidden_tile(h - LAG)

    loop(LAG, HQ - 1, v_even)
    loop(0, LAG, lambda h: kv_burst(vt_hbm, h, 1))

    def out_proj(o, h):
        return jnp.dot(o, wo_v[pl.ds(pl.multiple_of(h * DH, 16), DH), :], preferred_element_type=F32)

    def values(h, carry):
        acc, o_prev = carry

        @pl.when(h < HQ - 1 - LAG)
        def _():
            kv_burst(vt_hbm, h + LAG, 1)

        t = h - (HQ - 1 - LAG)
        for part in range(2):
            @pl.when((t >> 1) == part)
            def _():
                last_burst(part, (t & 1) * BURST)

        @pl.when(h == HQ - 1)
        def _():
            ffn[...] = consume_w2(0, W2_EARLY, ffn[...])

        wait_all(kv.at[h], kv_sem.at[h])
        o = lax.dot_general(p_all[h], kv[h], (((1,), (1,)), ((), ())), preferred_element_type=F32)
        return acc + out_proj(o_prev, jnp.maximum(h - 1, 0)), o.astype(BF16)

    attn, o_last = lax.fori_loop(0, HQ, values,
                                 (jnp.zeros((8, d_model), F32), jnp.zeros((8, DH), BF16)))
    attn = attn + out_proj(o_last, HQ - 1)

    tot = consume_w2(W2_EARLY, n_w2, ffn[...] + jnp.where(row0, gate * attn, 0.0))
    out_ref[0] = jnp.sum(tot, axis=0, keepdims=True).astype(out_ref.dtype)


def _compiler_params():
    params = dict(vmem_limit_bytes=96 * 1024 * 1024, disable_bounds_checks=True)
    try:
        return pltpu.CompilerParams(disable_semaphore_checks=True, **params)
    except TypeError:
        return pltpu.CompilerParams(**params)


@jax.jit
def pallas_gated_mix__sliding_block_cached__dense_activation_gelu__decode_kernel(
    A_x: jax.Array,
    A_k_cache: jax.Array,
    A_v_cache: jax.Array,
    A_wq: jax.Array,
    A_wo: jax.Array,
    B_x: jax.Array,
    B_w1: jax.Array,
    B_b1: jax.Array,
    B_w2: jax.Array,
    B_b2: jax.Array,
    gate_w: jax.Array,
):
    del B_x
    b, sq, d_model = A_x.shape
    _, hkv, sk, dh = A_k_cache.shape
    d_ff = B_w1.shape[1]
    win = min(4096, max(256, sk // 4))
    assert (b, sq, d_model, d_ff, hkv, dh, win) == (1, 1, 640, 1536, HQ, DH, 4096)
    kt = jnp.swapaxes(A_k_cache, 2, 3).reshape(HQ * DH, sk)
    vt = jnp.swapaxes(A_v_cache, 2, 3).reshape(HQ * DH, sk)

    any_spec = pl.BlockSpec(memory_space=pl.ANY)
    dma = pltpu.SemaphoreType.DMA
    return pl.pallas_call(
        functools.partial(_kernel, sk=sk, win=win),
        out_shape=jax.ShapeDtypeStruct((b, sq, d_model), A_x.dtype),
        in_specs=[any_spec] * 10,
        out_specs=pl.BlockSpec(memory_space=pltpu.VMEM),
        scratch_shapes=[
            pltpu.VMEM((HQ, DH, win), BF16),
            pltpu.VMEM((HQ, 8, win), BF16),
            pltpu.VMEM(A_wq.shape, BF16),
            pltpu.VMEM(A_wo.shape, BF16),
            pltpu.VMEM(B_w1.shape, BF16),
            pltpu.VMEM(B_w2.shape, BF16),
            pltpu.VMEM((d_ff, 128), F32),
            pltpu.VMEM((HQ, M, DH), BF16),
            pltpu.VMEM((8, d_model), F32),
            pltpu.VMEM((M, d_model), BF16),
            pltpu.VMEM((1, d_ff), F32),
            pltpu.VMEM(A_x.shape, BF16),
            pltpu.VMEM(gate_w.shape, BF16),
            pltpu.VMEM(B_b1.shape, BF16),
            pltpu.VMEM(B_b2.shape, BF16),
            dma((7,)), dma((d_ff // W2_ROWS,)), dma((HQ,)),
        ],
        compiler_params=_compiler_params(),
    )(A_x, kt, vt, A_wq, A_wo, B_w1, B_b1, B_w2, B_b2, gate_w)
```
